```python
import os as _os
_os.environ.setdefault("JAX_PLATFORMS", "cpu")
import jax
import jax.numpy as jnp

def _softmax(x, axis=-1):
    return jax.nn.softmax(x, axis=axis)
def _gelu(x):
    return jax.nn.gelu(x, approximate=True)
def _silu(x):
    return jax.nn.silu(x)
def _sigmoid(x):
    return jax.nn.sigmoid(x)
def _layernorm(x, axis=-1, eps=1e-5):
    m = jnp.mean(x, axis=axis, keepdims=True)
    v = jnp.var(x, axis=axis, keepdims=True)
    return (x - m) / jnp.sqrt(v + eps)
def _scatter_add(tgt, idx, src, axis=0):
    return tgt.at[idx].add(src)
def _segment_sum(src, seg, n):
    return jax.ops.segment_sum(src, seg, n)
class _Rng:
    def __init__(self, key):
        self._k = key
    def _next(self):
        self._k, sub = jax.random.split(self._k)
        return sub
    def normal(self, shape):
        return jax.random.normal(self._next(), shape, dtype=jnp.bfloat16)
    def randint(self, lo, hi, shape):
        return jax.random.randint(self._next(), shape, lo, hi, dtype=jnp.int32)
    def uniform(self, shape, lo=0.0, hi=1.0):
        return jax.random.uniform(self._next(), shape, jnp.bfloat16, lo, hi)
    def permutation(self, n):
        return jax.random.permutation(self._next(), n)


kernel_name = 'standalone__moe_arch_mod__prompt'

def setup_inputs():
    _rng = _Rng(jax.random.key(int.from_bytes(__import__("os").urandom(4), "little")))
    _w = (lambda a: (lambda t: t.astype(jnp.bfloat16) if jnp.issubdtype(t.dtype, jnp.floating) else t)(jnp.asarray(a)))
    B, S, D, F, C = 1, 2048, 576, 4608, 8
    return {
        "x": _w((lambda *s: _rng.normal(s) * 0.1)(B, S, D)),
        "w_r": _w((lambda *s: _rng.normal(s) * 0.1)(D)),
        "w_gate": _w((lambda *s: _rng.normal(s) * 0.1)(D, F)),
        "w_up": _w((lambda *s: _rng.normal(s) * 0.1)(D, F)),
        "w_down": _w((lambda *s: _rng.normal(s) * 0.1)(F, D)),
    }

def reference(x, w_r, w_gate, w_up, w_down):
    B, S, D = x.shape
    C = 8
    r = x @ w_r
    idx = jnp.argsort(-r, axis=-1)[:, :C]
    idx_e = jnp.repeat(idx.reshape(B, C, 1), D, axis=2)
    x_sel = jnp.take_along_axis(x, idx_e, axis=1)
    g = _silu(x_sel @ w_gate)
    u = x_sel @ w_up
    y = (g * u) @ w_down
    r_sel = _sigmoid(jnp.take_along_axis(r, idx, axis=1))
    y = y * r_sel.reshape(B, C, 1)
    b_off = (jnp.arange(B) * S).reshape(B, 1)
    flat_idx = (idx + b_off).reshape(B * C)
    zero = (x * 0.0).reshape(B * S, D)
    upd = _scatter_add(zero, flat_idx, y.reshape(B * C, D), axis=0)
    return x + upd.reshape(B, S, D)
```

```python
import functools

import jax
import jax.numpy as jnp
from jax import lax
import jax.experimental.pallas as pl
import jax.experimental.pallas.tpu as pltpu

C = 8
LANES = 128


def _kernel(x_hbm, wr_hbm, wg_hbm, wu_hbm, wd_hbm, o_hbm,
            xv, wrv, gv, uv, dv, ov, rsem, wsem, *, chunk, last, down_form, unroll):
    D, S = xv.shape
    F = gv.shape[1]
    n_tiles = S // LANES
    n_chunks = F // chunk
    f32, bf16, i32 = jnp.float32, jnp.bfloat16, jnp.int32

    x_cp = pltpu.make_async_copy(x_hbm, xv, rsem.at[0])
    wr_cp = pltpu.make_async_copy(wr_hbm, wrv, rsem.at[1])

    def w_copies(c):
        off = c * chunk if isinstance(c, int) else pl.multiple_of(c * chunk, LANES)
        sl = (slice(None), pl.ds(off, chunk))
        return (pltpu.make_async_copy(wg_hbm.at[sl], gv.at[sl], rsem.at[2 + 3 * c]),
                pltpu.make_async_copy(wu_hbm.at[sl], uv.at[sl], rsem.at[3 + 3 * c]),
                pltpu.make_async_copy(wd_hbm.at[sl], dv.at[sl], rsem.at[4 + 3 * c]))

    x_cp.start()
    wr_cp.start()
    for c in range(n_chunks - 1):
        for cp in w_copies(c):
            cp.start()
    lg, lu, _ = w_copies(n_chunks - 1)
    lg.start()
    lu.start()
    a0 = (n_chunks - 1) * chunk
    sl_a = (slice(None), pl.ds(a0, chunk - last))
    sl_b = (slice(None), pl.ds(F - last, last))
    if chunk > last:
        ld_a = pltpu.make_async_copy(wd_hbm.at[sl_a], dv.at[sl_a], rsem.at[4 + 3 * (n_chunks - 1)])
        ld_a.start()
    ld_b = pltpu.make_async_copy(wd_hbm.at[sl_b], dv.at[sl_b], rsem.at[5 + 3 * (n_chunks - 1)])
    ld_b.start()

    x_cp.wait()
    wr_cp.wait()
    wr = jnp.broadcast_to(wrv[...].astype(f32).reshape(1, D), (8, D)).astype(bf16)
    r_all = jnp.dot(wr, xv[...], preferred_element_type=f32)
    row = lax.broadcasted_iota(i32, (8, LANES), 0)
    lane = lax.broadcasted_iota(i32, (8, LANES), 1)
    keys = []
    for h in range(n_tiles // 8):
        r = r_all[:, h * 8 * LANES:(h * 8 + 1) * LANES]
        for t in range(1, 8):
            c0 = (h * 8 + t) * LANES
            r = jnp.where(row == t, r_all[:, c0:c0 + LANES], r)
        r = r.astype(bf16).astype(f32)
        r = jnp.where(r == 0.0, 0.0, r)
        u = lax.shift_right_logical(lax.bitcast_convert_type(r, i32), 16)
        s = jnp.where(u >= 0x8000, 0xFFFF - u, u + 0x8000)
        s = jnp.where(r != r, 0, s)
        tok = (h * 8 + row) * LANES + lane
        keys.append(lax.bitcast_convert_type(0x30000000 + s * S + (S - 1 - tok), f32))

    toks = []
    sel_key = jnp.zeros((8, LANES), i32)
    for j in range(C):
        m = functools.reduce(jnp.maximum, keys)
        m = jnp.max(jnp.max(m, axis=0, keepdims=True), axis=1, keepdims=True)
        keys = [jnp.where(k == m, 0.0, k) for k in keys]
        mi = lax.bitcast_convert_type(jnp.broadcast_to(m, (8, LANES)), i32) - 0x30000000
        sel_key = jnp.where((lane if down_form == "T" else row) == j, mi, sel_key)
        toks.append(S - 1 - (mi[0, 0] & (S - 1)))
    s = lax.shift_right_logical(sel_key, S.bit_length() - 1)
    u = jnp.where(s >= 0x8000, s - 0x8000, 0xFFFF - s)
    r_sel = lax.bitcast_convert_type(lax.shift_left(u, 16), f32)
    gate = jax.nn.sigmoid(r_sel).astype(bf16).astype(f32)

    lane_w = lax.broadcasted_iota(i32, (D // 2, LANES), 1)
    x_selT = jnp.zeros((D // 2, LANES), i32)
    offs = [pl.multiple_of((t // LANES) * LANES, LANES) for t in toks]
    for j in range(C):
        tile = pltpu.bitcast(xv[:, pl.ds(offs[j], LANES)], i32)
        tile = pltpu.roll(tile, (j - toks[j]) & (LANES - 1), 1)
        x_selT = jnp.where(lane_w == j, tile, x_selT)
    x_selT = pltpu.bitcast(x_selT, bf16)
    x_selT32 = x_selT.astype(f32)
    pad = -D % LANES
    x_sel32 = jnp.concatenate([x_selT32, jnp.zeros((pad, LANES), f32)], axis=0).T
    x_sel = x_sel32[:8, :D].astype(bf16)

    xs = xv[...].astype(f32)
    ov[...] = (xs + xs * 0.0).astype(bf16)

    def hidden(sl):
        g = jnp.dot(x_sel, gv[:, sl], preferred_element_type=f32).astype(bf16).astype(f32)
        u = jnp.dot(x_sel, uv[:, sl], preferred_element_type=f32).astype(bf16).astype(f32)
        a = jax.nn.silu(g).astype(bf16).astype(f32)
        return (a * u).astype(bf16)

    def down(h, sl):
        if down_form == "NT":
            return lax.dot_general(h, dv[:, sl], (((1,), (1,)), ((), ())), preferred_element_type=f32)
        hp = jnp.concatenate([h.astype(f32), jnp.zeros((LANES - 8, h.shape[1]), f32)], axis=0)
        return jnp.dot(dv[:, sl], hp.T.astype(bf16), preferred_element_type=f32)

    def step(c, y):
        cg, cu, cd = w_copies(c)
        off = c * chunk if isinstance(c, int) else pl.multiple_of(c * chunk, LANES)
        sl = pl.ds(off, chunk)
        cg.wait()
        cu.wait()
        h = hidden(sl)
        cd.wait()
        return y + down(h, sl)

    y = jnp.zeros((8, D) if down_form == "NT" else (D, LANES), f32)
    if unroll:
        for c in range(n_chunks - 1):
            y = step(c, y)
    else:
        y = lax.fori_loop(0, n_chunks - 1, step, y)

    hit = functools.reduce(lambda a, b: a | b, [lax.shift_left(1, t // LANES) for t in toks])

    def out_copy(i):
        sl = (slice(None), pl.ds(i * LANES, LANES))
        return pltpu.make_async_copy(ov.at[sl], o_hbm.at[sl], wsem)

    order = [(5 * i) % n_tiles for i in range(n_tiles)]

    def write_tiles(want):
        for i in order:
            pl.when(((hit >> i) & 1) == want)(out_copy(i).start)

    lg.wait()
    lu.wait()
    if chunk > last:
        h = hidden(pl.ds(a0, chunk))
        ld_a.wait()
        write_tiles(0)
        y = y + down(h[:, :chunk - last], pl.ds(a0, chunk - last))
    else:
        write_tiles(0)
        h = hidden(pl.ds(a0, chunk))
    ld_b.wait()
    y = y + down(h[:, chunk - last:], pl.ds(F - last, last))

    if down_form == "NT":
        y = y.astype(bf16).astype(f32) * gate[:, :1]
        y = y.astype(bf16).astype(f32)
        xs = x_sel.astype(f32)
        o_sel = xs + (xs * 0.0 + y)
        o_sel = jnp.concatenate([o_sel, jnp.zeros((8, pad), f32)], axis=1)
        o_sel = jnp.concatenate([o_sel, jnp.zeros((LANES - 8, D + pad), f32)], axis=0)
        o_selT = o_sel.T[:D].astype(bf16)
    else:
        y = y.astype(bf16).astype(f32) * gate[:1, :]
        y = y.astype(bf16).astype(f32)
        o_selT = (x_selT32 + (x_selT32 * 0.0 + y)).astype(bf16)
    o_selT = pltpu.bitcast(o_selT, i32)
    for j in range(C):
        sl = pl.ds(offs[j], LANES)
        tile = pltpu.bitcast(ov[:, sl], i32)
        new = pltpu.roll(o_selT, (toks[j] - j) & (LANES - 1), 1)
        tile = jnp.where(lane_w == (toks[j] & (LANES - 1)), new, tile)
        ov[:, sl] = pltpu.bitcast(tile, bf16)
    write_tiles(1)
    pltpu.make_async_copy(ov, o_hbm, wsem).wait()


def make(chunk=512, last=256, down_form="NT", unroll=False, **cp):
    def f(x, w_r, w_gate, w_up, w_down):
        B, S, D = x.shape
        F = w_gate.shape[1]
        xT = x.reshape(S, D).T
        hbm = pl.BlockSpec(memory_space=pltpu.HBM)
        params = dict(vmem_limit_bytes=64 * 1024 * 1024, disable_semaphore_checks=True)
        params.update(cp)
        oT = pl.pallas_call(
            functools.partial(_kernel, chunk=chunk, last=last, down_form=down_form, unroll=unroll),
            out_shape=jax.ShapeDtypeStruct((D, S), x.dtype),
            in_specs=[hbm] * 5,
            out_specs=hbm,
            scratch_shapes=[
                pltpu.VMEM((D, S), x.dtype),
                pltpu.VMEM((D,), x.dtype),
                pltpu.VMEM((D, F), x.dtype),
                pltpu.VMEM((D, F), x.dtype),
                pltpu.VMEM((D, F), x.dtype),
                pltpu.VMEM((D, S), x.dtype),
                pltpu.SemaphoreType.DMA((3 + 3 * (F // chunk),)),
                pltpu.SemaphoreType.DMA,
            ],
            compiler_params=pltpu.CompilerParams(**params),
        )(xT, w_r, w_gate, w_up, w_down.T)
        return oT.T.reshape(B, S, D)
    return f


@jax.jit
def pallas_standalone__moe_arch_mod__prompt_kernel(x, w_r, w_gate, w_up, w_down):
    return make(chunk=1152, last=256, down_form="NT", unroll=True)(x, w_r, w_gate, w_up, w_down)
```

```python
import functools

import jax
import jax.numpy as jnp
from jax import lax
import jax.experimental.pallas as pl
import jax.experimental.pallas.tpu as pltpu

CAPACITY = 8
LANES = 128
TILE_ROWS = 8
GROUPS = 4

BLOCK = 512
STEP_BLOCKS = 8
DEPTH = 13
RING = 22
WRITE_LEAD = 7
READ_PITCH = 64
WRITE_PITCH = 19


def _interleaved(n, pitch):
    return [i for start in range(pitch) for i in range(start, n, pitch)]


def _interleaved_rows(n, pitch, row):
    starts = [min(-(-s // row) * row, n) for s in range(0, n + pitch, pitch)]
    return [j * pitch + t for t in range(pitch + row) for j in range(len(starts) - 1)
            if starts[j] <= j * pitch + t < starts[j + 1]]


class _ReadStream:
    def __init__(self, sems):
        self.sems = sems
        self.steps = []
        self.issued = 0
        self.retired = 0
        self.on_retire = {}

    def add(self, src, dst, order):
        for k in range(0, len(order), STEP_BLOCKS):
            sem = self.sems.at[len(self.steps) % RING]
            step = []
            for block in order[k:k + STEP_BLOCKS]:
                tile_row, col = divmod(block, src.shape[1] // BLOCK)
                step.append(pltpu.make_async_copy(
                    src.at[pl.ds(tile_row * TILE_ROWS, TILE_ROWS), pl.ds(col * BLOCK, BLOCK)],
                    dst(tile_row, col), sem))
            self.steps.append(step)
        return len(self.steps)

    def issue(self):
        if self.issued < len(self.steps):
            assert self.issued - RING < self.retired
            for i, copy in enumerate(self.steps[self.issued]):
                copy.start(priority=int(i > 0))
        self.issued += 1

    def sync(self):
        while self.retired < min(self.issued - DEPTH + 1, len(self.steps)):
            for copy in self.steps[self.retired]:
                copy.wait()
            self.retired += 1
            if self.retired in self.on_retire:
                self.on_retire[self.retired]()

    def advance(self, n):
        for _ in range(n):
            self.sync()
            self.issue()

    def wait_for(self, n_steps):
        while self.retired < n_steps:
            self.advance(1)

    def interleave(self, items, work, sync_every):
        for i, item in enumerate(items):
            if i % sync_every == 0:
                self.sync()
            work(*item)
            self.issue()


def _mod_kernel(x_hbm, wr_hbm, wg_hbm, wu_hbm, wd_hbm, o_hbm,
                buf, out_ref, wr_ref, key_ref, xt_ref, xs_ref, a_ref, h_ref, y_ref, z_ref,
                read_sems, wr_sem, write_sem):
    D, S = x_hbm.shape
    F = wg_hbm.shape[1]
    n_rows, n_feat = D // TILE_ROWS, D // GROUPS
    x_blocks, w_blocks = S // BLOCK, F // BLOCK
    X, WG, WU, WD = 0, x_blocks, x_blocks + w_blocks, x_blocks + 2 * w_blocks
    f32, bf16, i32 = jnp.float32, jnp.bfloat16, jnp.int32

    def round_bf16(v):
        return v.astype(bf16).astype(f32)

    def half_blocks(n):
        return [(b, c) for b in range(n) for c in (0, BLOCK // 2)]

    wd_order = _interleaved_rows(n_rows * w_blocks, READ_PITCH, w_blocks)
    last_block = {block // w_blocks: i for i, block in enumerate(wd_order)}
    tile_rows = sorted(range(n_rows), key=last_block.get)
    staged_row = {tile_row: p * TILE_ROWS for p, tile_row in enumerate(tile_rows)}

    def stage_at(first):
        return lambda tile_row, col: buf.at[first + col, pl.ds(staged_row[tile_row], TILE_ROWS)]

    stream = _ReadStream(read_sems)
    x_end = stream.add(x_hbm, stage_at(X), _interleaved(n_rows * x_blocks, READ_PITCH))
    wg_end = stream.add(wg_hbm, stage_at(WG), _interleaved(n_rows * w_blocks, READ_PITCH))
    wu_end = stream.add(wu_hbm, stage_at(WU), _interleaved(n_rows * w_blocks, READ_PITCH))
    wd_end = stream.add(wd_hbm, stage_at(WD), wd_order)
    group_end = [wu_end + last_block[tile_rows[(m + 1) * n_rows // GROUPS - 1]] // STEP_BLOCKS + 1
                 for m in range(GROUPS)]
    assert group_end[-1] == wd_end

    final_groups = []

    def write_final_groups():
        for tile_row in _interleaved(n_rows, WRITE_PITCH):
            if staged_row[tile_row] // n_feat in final_groups:
                pltpu.make_async_copy(out_ref.at[pl.ds(staged_row[tile_row], TILE_ROWS)],
                                      o_hbm.at[pl.ds(tile_row * TILE_ROWS, TILE_ROWS)],
                                      write_sem).start()
        final_groups.clear()

    write_start = wd_end - WRITE_LEAD
    stream.on_retire[write_start] = write_final_groups

    def keep_write_start_on_time(steps):
        if stream.retired < write_start <= stream.retired + steps:
            stream.wait_for(write_start)

    wr_copy = pltpu.make_async_copy(wr_hbm, wr_ref, wr_sem)
    stream.issue()
    wr_copy.start()
    for _ in range(DEPTH - 1):
        stream.issue()

    stream.advance(8)
    wr_copy.wait()
    wr = jnp.broadcast_to(wr_ref[...].astype(f32).reshape(1, D), (8, D))
    xs_ref[...] = jnp.concatenate(
        [wr[:, r * TILE_ROWS:(r + 1) * TILE_ROWS] for r in tile_rows], axis=1).astype(bf16)
    stream.wait_for(x_end)
    wr = xs_ref[...]
    scores = []

    def score(b, c):
        scores.append(jnp.dot(wr, buf[X + b, :, c:c + BLOCK // 2], preferred_element_type=f32))

    stream.interleave(half_blocks(x_blocks), score, 8)
    scores = jnp.concatenate(scores, axis=1)

    row = lax.broadcasted_iota(i32, (8, LANES), 0)
    lane = lax.broadcasted_iota(i32, (8, LANES), 1)
    key_base = 0x30000000
    for i in range(S // (8 * LANES)):
        r = scores[:, i * 8 * LANES:(i * 8 + 1) * LANES]
        for t in range(1, 8):
            c = (i * 8 + t) * LANES
            r = jnp.where(row == t, scores[:, c:c + LANES], r)
        bits = lax.shift_right_logical(lax.bitcast_convert_type(round_bf16(r), i32), 16)
        bits = jnp.where(bits == 0x8000, 0, bits)
        rank = jnp.where(bits >= 0x8000, 0xFFFF - bits, bits + 0x8000)
        rank = jnp.where((bits & 0x7FFF) > 0x7F80, 0, rank)
        token = (i * 8 + row) * LANES + lane
        key_ref[i] = lax.bitcast_convert_type(key_base + rank * S + (S - 1 - token), f32)
    stream.advance(1)

    tokens = []
    top_keys = jnp.zeros((8, LANES), i32)
    for j in range(CAPACITY):
        keys = key_ref[...]
        best = jnp.max(jnp.max(jnp.max(keys, axis=0), axis=0, keepdims=True), axis=1, keepdims=True)
        key_ref[...] = jnp.where(keys == best, 0.0, keys)
        best = lax.bitcast_convert_type(jnp.broadcast_to(best, (8, LANES)), i32) - key_base
        top_keys = jnp.where(row == j, best, top_keys)
        tokens.append(S - 1 - (best[0, 0] & (S - 1)))
        stream.advance(1 if j % 3 == 2 else 2)
    rank = lax.shift_right_logical(top_keys, S.bit_length() - 1)
    bits = jnp.where(rank >= 0x8000, rank - 0x8000, 0xFFFF - rank)
    top_scores = lax.bitcast_convert_type(lax.shift_left(bits, 16), f32)
    router_weight = round_bf16(jax.nn.sigmoid(top_scores))[:, :1]

    lane_ids = lax.broadcasted_iota(i32, (D // 2, LANES), 1)
    picked = [jnp.zeros((D // 2, LANES), i32)]

    def gather(j):
        block = X + lax.shift_right_logical(tokens[j], BLOCK.bit_length() - 1)
        cols = pl.ds(pl.multiple_of(tokens[j] & (BLOCK - LANES), LANES), LANES)
        tile = pltpu.bitcast(buf[block, :, cols], i32)
        tile = pltpu.roll(tile, (j - tokens[j]) & (LANES - 1), 1)
        picked[0] = jnp.where(lane_ids == j, tile, picked[0])

    stream.interleave([(j,) for j in range(CAPACITY)], gather, CAPACITY)
    x_sel_t = pltpu.bitcast(picked[0], bf16).astype(f32)
    xt_ref[...] = x_sel_t
    x_sel = jnp.concatenate([x_sel_t, jnp.zeros((-D % LANES, LANES), f32)], axis=0).T
    xs_ref[...] = x_sel[:CAPACITY, :D].astype(bf16)
    stream.advance(2)

    def residual(b, r):
        x = buf[X + b, r:r + D // 2, :].astype(f32)
        out_ref[r:r + D // 2, b * BLOCK:(b + 1) * BLOCK] = (x + x * 0.0).astype(bf16)

    stream.interleave([(b, r) for b in range(x_blocks) for r in (0, D // 2)], residual, 1)

    def gate_proj(b, c):
        cols = pl.ds(b * BLOCK + c, BLOCK // 2)
        g = jnp.dot(xs_ref[...], buf[WG + b, :, c:c + BLOCK // 2], preferred_element_type=f32)
        a_ref[:, cols] = round_bf16(jax.nn.silu(round_bf16(g)))

    def up_proj(b, c):
        cols = pl.ds(b * BLOCK + c, BLOCK // 2)
        u = jnp.dot(xs_ref[...], buf[WU + b, :, c:c + BLOCK // 2], preferred_element_type=f32)
        h_ref[:, cols] = (a_ref[:, cols] * round_bf16(u)).astype(bf16)

    stream.wait_for(wg_end)
    stream.interleave(half_blocks(w_blocks), gate_proj, 6)
    stream.wait_for(wu_end)
    stream.interleave(half_blocks(w_blocks), up_proj, 6)

    group_lane_ids = lax.broadcasted_iota(i32, (n_feat // 2, LANES), 1)
    for m in range(GROUPS):
        rows = pl.ds(m * n_feat, n_feat)
        partial = []

        def down_proj(b):
            partial.append(lax.dot_general(h_ref[:, b * BLOCK:(b + 1) * BLOCK], buf[WD + b, rows, :],
                                           (((1,), (1,)), ((), ())), preferred_element_type=f32))

        stream.wait_for(group_end[m])
        stream.interleave([(b,) for b in range(w_blocks)], down_proj, w_blocks)
        y_ref[...] = functools.reduce(jnp.add, partial)
        stream.advance(1)
        keep_write_start_on_time(2)

        y = round_bf16(round_bf16(y_ref[...]) * router_weight)
        y = jnp.concatenate([y, jnp.zeros((CAPACITY, -n_feat % LANES), f32)], axis=1)
        y = jnp.concatenate([y, jnp.zeros((LANES - CAPACITY, y.shape[1]), f32)], axis=0)
        x = xt_ref[rows, :]
        z_ref[...] = pltpu.bitcast((x + (x * 0.0 + y.T[:n_feat])).astype(bf16), i32)
        stream.advance(2)
        keep_write_start_on_time(5)

        z = z_ref[...]

        def scatter(*js):
            for j in js:
                new = pltpu.roll(z, (tokens[j] - j) & (LANES - 1), 1)
                cols = pl.ds(pl.multiple_of(tokens[j] & (S - LANES), LANES), LANES)
                tile = pltpu.bitcast(out_ref[rows, cols], i32)
                tile = jnp.where(group_lane_ids == (tokens[j] & (LANES - 1)), new, tile)
                out_ref[rows, cols] = pltpu.bitcast(tile, bf16)

        stream.interleave([(j, j + 1) for j in range(0, CAPACITY, 2)], scatter, CAPACITY)
        final_groups.append(m)
        if stream.retired >= write_start:
            write_final_groups()

    assert stream.retired == wd_end and not final_groups
    pltpu.make_async_copy(o_hbm, o_hbm, write_sem).wait()


@jax.jit
def pallas_standalone__moe_arch_mod__prompt_kernel(
    x: jax.Array,
    w_r: jax.Array,
    w_gate: jax.Array,
    w_up: jax.Array,
    w_down: jax.Array,
):
    B, S, D = x.shape
    F = w_gate.shape[1]
    assert B == 1 and S in (1024, 2048) and D % (16 * GROUPS) == 0 and F % BLOCK == 0
    n_feat = D // GROUPS
    hbm = pl.BlockSpec(memory_space=pltpu.HBM)
    out_t = pl.pallas_call(
        _mod_kernel,
        out_shape=jax.ShapeDtypeStruct((D, S), x.dtype),
        in_specs=[hbm] * 5,
        out_specs=hbm,
        scratch_shapes=[
            pltpu.VMEM(((S + 3 * F) // BLOCK, D, BLOCK), x.dtype),
            pltpu.VMEM((D, S), x.dtype),
            pltpu.VMEM((D,), w_r.dtype),
            pltpu.VMEM((S // (8 * LANES), 8, LANES), jnp.float32),
            pltpu.VMEM((D, LANES), jnp.float32),
            pltpu.VMEM((CAPACITY, D), x.dtype),
            pltpu.VMEM((CAPACITY, F), jnp.float32),
            pltpu.VMEM((CAPACITY, F), x.dtype),
            pltpu.VMEM((CAPACITY, n_feat), jnp.float32),
            pltpu.VMEM((n_feat // 2, LANES), jnp.int32),
            pltpu.SemaphoreType.DMA((RING,)),
            pltpu.SemaphoreType.DMA,
            pltpu.SemaphoreType.DMA,
        ],
        compiler_params=pltpu.CompilerParams(
            vmem_limit_bytes=64 * 1024 * 1024,
            disable_semaphore_checks=True,
        ),
    )(x.reshape(S, D).T, w_r, w_gate, w_up, w_down.T)
    return out_t.T.reshape(B, S, D)
```
